```python
import jax
import jax.numpy as jnp

def _softmax(x, axis=-1):
    return jax.nn.softmax(x, axis=axis)
def _gelu(x):
    return jax.nn.gelu(x, approximate=True)
def _silu(x):
    return jax.nn.silu(x)
def _sigmoid(x):
    return jax.nn.sigmoid(x)
def _layernorm(x, axis=-1, eps=1e-5):
    m = jnp.mean(x, axis=axis, keepdims=True)
    v = jnp.var(x, axis=axis, keepdims=True)
    return (x - m) / jnp.sqrt(v + eps)
def _scatter_add(tgt, idx, src, axis=0):
    return tgt.at[idx].add(src)
def _segment_sum(src, seg, n):
    return jax.ops.segment_sum(src, seg, n)
class _Rng:
    def __init__(self, key):
        self._k = key
    def _next(self):
        self._k, sub = jax.random.split(self._k)
        return sub
    def normal(self, shape):
        return jax.random.normal(self._next(), shape, dtype=jnp.bfloat16)
    def randint(self, lo, hi, shape):
        return jax.random.randint(self._next(), shape, lo, hi, dtype=jnp.int32)
    def uniform(self, shape, lo=0.0, hi=1.0):
        return jax.random.uniform(self._next(), shape, jnp.bfloat16, lo, hi)
    def permutation(self, n):
        return jax.random.permutation(self._next(), n)


kernel_name = 'sequential_preLN__sliding_block_cached__moe_arch_mod__decode'

def setup_inputs():
    _rng = _Rng(jax.random.key(int.from_bytes(__import__("os").urandom(4), "little")))
    _w = (lambda a: (lambda t: t.astype(jnp.bfloat16) if jnp.issubdtype(t.dtype, jnp.floating) else t)(jnp.asarray(a)))
    def _A_setup():
        B, Sq, D = 1, 1, 640
        Hq, Hkv, Sk, Dh = 32, 32, 32768, 192
        assert Hq % Hkv == 0, (Hq, Hkv)
        return {
            "x": _w((lambda *s: _rng.normal(s) * 0.05)(B, Sq, D)),
            "k_cache": _w((lambda *s: _rng.normal(s) * 0.05)(B, Hkv, Sk, Dh)),
            "v_cache": _w((lambda *s: _rng.normal(s) * 0.05)(B, Hkv, Sk, Dh)),
            "wq": _w((lambda *s: _rng.normal(s) * 0.05)(D, Hq * Dh) * (D ** -0.5)),
            "wo": _w((lambda *s: _rng.normal(s) * 0.05)(Hq * Dh, D) * ((Hq * Dh) ** -0.5)),
        }
    _A_in = _A_setup()

    def _B_setup():
        B, S, D, F, C = 1, 1, 640, 1536, 1
        return {
            "x": _w((lambda *s: _rng.normal(s) * 0.05)(B, S, D)),
            "w_r": _w((lambda *s: _rng.normal(s) * 0.05)(D)),
            "w_gate": _w((lambda *s: _rng.normal(s) * 0.05)(D, F)),
            "w_up": _w((lambda *s: _rng.normal(s) * 0.05)(D, F)),
            "w_down": _w((lambda *s: _rng.normal(s) * 0.05)(F, D)),
        }
    _B_in = _B_setup()

    return {
        "A_x": _A_in["x"],
        "A_k_cache": _A_in["k_cache"],
        "A_v_cache": _A_in["v_cache"],
        "A_wq": _A_in["wq"],
        "A_wo": _A_in["wo"],
        "B_x": _B_in["x"],
        "B_w_r": _B_in["w_r"],
        "B_w_gate": _B_in["w_gate"],
        "B_w_up": _B_in["w_up"],
        "B_w_down": _B_in["w_down"],
    }

def reference(A_x, A_k_cache, A_v_cache, A_wq, A_wo, B_x, B_w_r, B_w_gate, B_w_up, B_w_down):
    def _A_ref(x, k_cache, v_cache, wq, wo):
        B, Sq, D = x.shape
        Hq, Dh = 32, 192
        Hkv, Sk = k_cache.shape[1], k_cache.shape[2]
        W = min(4096, max(256, Sk // 4))
        rep = Hq // Hkv
        q = (lambda x, *d: x.transpose(*d))((x @ wq).reshape(B, Sq, Hq, Dh), 0, 2, 1, 3)
        k = jnp.repeat(k_cache[:, :, Sk - W:, :], rep, axis=1)
        v = jnp.repeat(v_cache[:, :, Sk - W:, :], rep, axis=1)
        scores = jnp.einsum("bhqd,bhkd->bhqk", q, k) * (Dh ** -0.5)
        p = _softmax(scores, axis=-1)
        o = jnp.einsum("bhqk,bhkd->bhqd", p, v)
        return (lambda x, *d: x.transpose(*d))(o, 0, 2, 1, 3).reshape(B, Sq, Hq * Dh) @ wo

    def _B_ref(x, w_r, w_gate, w_up, w_down):
        B, S, D = x.shape
        C = 1
        r = x @ w_r
        idx = jnp.argsort(-r, axis=-1)[:, :C]
        idx_e = jnp.repeat(idx.reshape(B, C, 1), D, axis=2)
        x_sel = jnp.take_along_axis(x, idx_e, axis=1)
        g = _silu(x_sel @ w_gate)
        u = x_sel @ w_up
        y = (g * u) @ w_down
        r_sel = _sigmoid(jnp.take_along_axis(r, idx, axis=1))
        y = y * r_sel.reshape(B, C, 1)
        b_off = (jnp.arange(B) * S).reshape(B, 1)
        flat_idx = (idx + b_off).reshape(B * C)
        zero = (x * 0.0).reshape(B * S, D)
        upd = _scatter_add(zero, flat_idx, y.reshape(B * C, D), axis=0)
        return x + upd.reshape(B, S, D)

    x = A_x
    h = x + _A_ref(_layernorm(x, axis=-1), A_k_cache, A_v_cache, A_wq, A_wo)
    h2 = h + _B_ref(_layernorm(h, axis=-1), B_w_r, B_w_gate, B_w_up, B_w_down)
    return h2
```

```python
import functools

import jax
import jax.numpy as jnp
import jax.experimental.pallas as pl
import jax.experimental.pallas.tpu as pltpu

_HQ, _DH = 32, 192
_EPS = 1e-5


def _layernorm(x):
    m = jnp.mean(x, axis=-1, keepdims=True)
    c = x - m
    v = jnp.mean(c * c, axis=-1, keepdims=True)
    return c / jnp.sqrt(v + _EPS)


def _kernel(x_hbm, kt_hbm, vt_hbm, wq_hbm, wo_hbm, wr_hbm, wg_hbm, wu_hbm, wd_hbm,
            out_ref,
            x_v, wr_v, wq_v, wo_v, wg_v, wu_v, wd_v, k_v, v_v, q_v,
            s_small, s_wq, s_k, s_v, s_wo, s_ffn,
            *, W, NS, NQ, ND):
    D = x_v.shape[-1]
    Sk = kt_hbm.shape[-1]
    F = wg_v.shape[-1]
    NP = _HQ // 2
    PR = 2 * _DH
    R = 16
    qr = D // NQ
    dr = F // ND
    f32, bf16 = jnp.float32, jnp.bfloat16

    def x_dma():
        return pltpu.make_async_copy(x_hbm, x_v, s_small.at[0])

    def wr_dma():
        return pltpu.make_async_copy(wr_hbm, wr_v, s_small.at[1])

    def wq_dma(i):
        return pltpu.make_async_copy(wq_hbm.at[pl.ds(i * qr, qr)], wq_v.at[pl.ds(i * qr, qr)], s_wq.at[i])

    def k_dma(j, slot):
        return pltpu.make_async_copy(kt_hbm.at[0, pl.ds(2 * j, 2), :, pl.ds(Sk - W, W)], k_v.at[slot], s_k.at[slot])

    def v_dma(j, slot):
        return pltpu.make_async_copy(vt_hbm.at[0, pl.ds(2 * j, 2), :, pl.ds(Sk - W, W)], v_v.at[slot], s_v.at[slot])

    def wo_dma(j):
        r0 = pl.multiple_of(j * PR, PR)
        return pltpu.make_async_copy(wo_hbm.at[pl.ds(r0, PR)], wo_v.at[pl.ds(r0, PR)], s_wo.at[j])

    def wg_dma():
        return pltpu.make_async_copy(wg_hbm, wg_v, s_ffn.at[0])

    def wu_dma():
        return pltpu.make_async_copy(wu_hbm, wu_v, s_ffn.at[1])

    def wd_dma(i):
        return pltpu.make_async_copy(wd_hbm.at[pl.ds(i * dr, dr)], wd_v.at[pl.ds(i * dr, dr)], s_ffn.at[2 + i])

    wq_dma(0).start()
    x_dma().start()
    for i in range(1, NQ):
        wq_dma(i).start()
    for j in range(NS):
        k_dma(j, j).start()
        v_dma(j, j).start()
        wo_dma(j).start()
    wr_dma().start()

    x_dma().wait()
    x = x_v[0].astype(f32)
    xn = jnp.broadcast_to(_layernorm(x), (R, D)).astype(bf16)
    q = None
    for i in range(NQ):
        wq_dma(i).wait()
        t = jnp.dot(xn[:, i * qr:(i + 1) * qr], wq_v[pl.ds(i * qr, qr), :], preferred_element_type=f32)
        q = t if q is None else q + t
    row = jax.lax.broadcasted_iota(jnp.int32, (R, PR), 0)
    col = jax.lax.broadcasted_iota(jnp.int32, (R, PR), 1)
    diag = row == jnp.where(col >= _DH, 1, 0)
    for j in range(NP):
        q_v[j] = jnp.where(diag, q[:, j * PR:(j + 1) * PR], 0.0).astype(bf16)

    late = [wg_dma, wu_dma] + [functools.partial(wd_dma, i) for i in range(ND)]

    def start_late(j, phase):
        for n, mk in enumerate(late):
            step = min(n, 2 * NS - 1)
            if step % 2 == phase:
                @pl.when(j == NP - NS + step // 2)
                def _():
                    mk().start()

    scale = _DH ** -0.5

    def pair(j, acc):
        slot = j % NS
        k_dma(j, slot).wait()
        s = jnp.dot(q_v[j], k_v[slot].reshape(PR, W), preferred_element_type=f32)[:8] * scale

        @pl.when(j + NS < NP)
        def _():
            k_dma(j + NS, slot).start()
        start_late(j, 0)

        m = jnp.max(s, axis=-1, keepdims=True)
        e = jnp.exp(s - m)
        p = e / jnp.sum(e, axis=-1, keepdims=True)
        p = jnp.concatenate([p, p], axis=0).astype(bf16)
        v_dma(j, slot).wait()
        o = jax.lax.dot_general(p, v_v[slot].reshape(PR, W), (((1,), (1,)), ((), ())),
                                preferred_element_type=f32)

        @pl.when(j + NS < NP)
        def _():
            v_dma(j + NS, slot).start()
            wo_dma(j + NS).start()
        start_late(j, 1)

        o = jnp.sum(jnp.where(diag, o, 0.0), axis=0, keepdims=True)
        o = jnp.broadcast_to(o, (R, PR)).astype(bf16)
        wo_dma(j).wait()
        wo = wo_v[pl.ds(pl.multiple_of(j * PR, PR), PR), :]
        return acc + jnp.dot(o, wo, preferred_element_type=f32)[:8]

    acc = jax.lax.fori_loop(0, NP, pair, jnp.zeros((8, D), f32))

    h = (x + acc[:1].astype(bf16).astype(f32)).astype(bf16).astype(f32)
    hn = _layernorm(h).astype(bf16)
    hn32 = hn.astype(f32)
    wr_dma().wait()
    r = jnp.sum(hn32 * wr_v[...].astype(f32).reshape(1, D), axis=-1, keepdims=True)
    hb = jnp.broadcast_to(hn32, (R, D)).astype(bf16)
    wg_dma().wait()
    g = jnp.dot(hb, wg_v[...], preferred_element_type=f32)
    wu_dma().wait()
    u = jnp.dot(hb, wu_v[...], preferred_element_type=f32)
    a = (jax.nn.silu(g) * u).astype(bf16)
    y = None
    for i in range(ND):
        wd_dma(i).wait()
        t = jnp.dot(a[:, i * dr:(i + 1) * dr], wd_v[pl.ds(i * dr, dr), :], preferred_element_type=f32)
        y = t if y is None else y + t
    y = y[:1] * jax.nn.sigmoid(r)
    out_ref[0] = (h + (hn32 + (hn32 * 0.0 + y))).astype(out_ref.dtype)


def _call(A_x, A_k_cache, A_v_cache, A_wq, A_wo, B_w_r, B_w_gate, B_w_up, B_w_down, NS=3, NQ=1, ND=6):
    _, _, D = A_x.shape
    Sk = A_k_cache.shape[2]
    F = B_w_gate.shape[1]
    W = min(4096, max(256, Sk // 4))
    kt = jnp.swapaxes(A_k_cache, 2, 3)
    vt = jnp.swapaxes(A_v_cache, 2, 3)
    bf16 = jnp.bfloat16
    hbm = pl.BlockSpec(memory_space=pltpu.HBM)
    return pl.pallas_call(
        functools.partial(_kernel, W=W, NS=NS, NQ=NQ, ND=ND),
        out_shape=jax.ShapeDtypeStruct(A_x.shape, A_x.dtype),
        in_specs=[hbm] * 9,
        out_specs=pl.BlockSpec(memory_space=pltpu.VMEM),
        scratch_shapes=[
            pltpu.VMEM(A_x.shape, bf16),
            pltpu.VMEM(B_w_r.shape, bf16),
            pltpu.VMEM(A_wq.shape, bf16),
            pltpu.VMEM(A_wo.shape, bf16),
            pltpu.VMEM(B_w_gate.shape, bf16),
            pltpu.VMEM(B_w_up.shape, bf16),
            pltpu.VMEM(B_w_down.shape, bf16),
            pltpu.VMEM((NS, 2, _DH, W), bf16),
            pltpu.VMEM((NS, 2, _DH, W), bf16),
            pltpu.VMEM((_HQ // 2, 16, 2 * _DH), bf16),
            pltpu.SemaphoreType.DMA((2,)),
            pltpu.SemaphoreType.DMA((NQ,)),
            pltpu.SemaphoreType.DMA((NS,)),
            pltpu.SemaphoreType.DMA((NS,)),
            pltpu.SemaphoreType.DMA((_HQ // 2,)),
            pltpu.SemaphoreType.DMA((2 + ND,)),
        ],
        compiler_params=pltpu.CompilerParams(vmem_limit_bytes=100 * 1024 * 1024),
    )(A_x, kt, vt, A_wq, A_wo, B_w_r, B_w_gate, B_w_up, B_w_down)


@jax.jit
def pallas_sequential_preLN__sliding_block_cached__moe_arch_mod__decode_kernel(
    A_x: jax.Array,
    A_k_cache: jax.Array,
    A_v_cache: jax.Array,
    A_wq: jax.Array,
    A_wo: jax.Array,
    B_x: jax.Array,
    B_w_r: jax.Array,
    B_w_gate: jax.Array,
    B_w_up: jax.Array,
    B_w_down: jax.Array,
):
    return _call(A_x, A_k_cache, A_v_cache, A_wq, A_wo, B_w_r, B_w_gate, B_w_up, B_w_down)
```
